```python
import os as _os
_os.environ.setdefault('JAX_PLATFORMS', 'cpu')
import jax
import jax.numpy as jnp

def _softmax(x, axis=-1):
    return jax.nn.softmax(x, axis=axis)

def _gelu(x):
    return jax.nn.gelu(x, approximate=True)

def _silu(x):
    return jax.nn.silu(x)

def _sigmoid(x):
    return jax.nn.sigmoid(x)

def _layernorm(x, axis=-1, eps=1e-05):
    m = jnp.mean(x, axis=axis, keepdims=True)
    v = jnp.var(x, axis=axis, keepdims=True)
    return (x - m) / jnp.sqrt(v + eps)

def _scatter_add(tgt, idx, src, axis=0):
    return tgt.at[idx].add(src)

def _segment_sum(src, seg, n):
    return jax.ops.segment_sum(src, seg, n)

class _Rng:

    def __init__(self, key):
        self._k = key

    def _next(self):
        self._k, sub = jax.random.split(self._k)
        return sub

    def normal(self, shape):
        return jax.random.normal(self._next(), shape, dtype=jnp.bfloat16)

    def randint(self, lo, hi, shape):
        return jax.random.randint(self._next(), shape, lo, hi, dtype=jnp.int32)

    def uniform(self, shape, lo=0.0, hi=1.0):
        return jax.random.uniform(self._next(), shape, jnp.bfloat16, lo, hi)

    def permutation(self, n):
        return jax.random.permutation(self._next(), n)
kernel_name = 'standalone__conformer_conv_module__speech'

def setup_inputs():
    _rng = _Rng(jax.random.key(int.from_bytes(__import__("os").urandom(4), "little")))
    _w = lambda a: (lambda t: t.astype(jnp.bfloat16) if jnp.issubdtype(t.dtype, jnp.floating) else t)(jnp.asarray(a))
    B, T, D, K = (2, 16000, 256, 5)
    return {'x': _w((lambda *s: _rng.normal(s) * 0.2)(B, T, D)), 'w_pw1': _w((lambda *s: _rng.normal(s) * 0.2)(D, 2 * D)), 'dw': _w((lambda *s: _rng.normal(s) * 0.05)(K, D)), 'w_pw2': _w((lambda *s: _rng.normal(s) * 0.05)(D, D))}

def reference(x, w_pw1, dw, w_pw2):
    B, T, D = x.shape
    K = dw.shape[0]
    h = x @ w_pw1
    a, b = (h[..., :D].copy(), h[..., D:].copy())
    h = a * _sigmoid(b)
    pad = K // 2
    hp = jnp.pad(h, ((0, 0), (pad, pad), (0, 0)))
    out = jnp.zeros_like(h)
    for i in range(K):
        out = out + hp[:, i:i + T, :] * dw[i][None, None, :]
    return _silu(out) @ w_pw2
```

```python
import jax
import jax.numpy as jnp
import jax.experimental.pallas as pl
import jax.experimental.pallas.tpu as pltpu

TT = 2000


def _kernel(x_ref, xn_ref, w1_ref, dw_ref, w2_ref, o_ref, h_ref, w1s_ref):
    b = pl.program_id(0)
    i = pl.program_id(1)
    n = pl.num_programs(1)
    D = 256

    @pl.when(jnp.logical_and(b == 0, i == 0))
    def _():
        w1s_ref[...] = (w1_ref[...].astype(jnp.float32) * 0.5).astype(jnp.bfloat16)

    @pl.when(i == 0)
    def _():
        h_ref[0:8, :] = jnp.zeros((8, D), jnp.float32)

    @pl.when(i > 0)
    def _():
        h_ref[0:8, :] = h_ref[TT:TT + 8, :]

    w1 = w1s_ref[...]

    def glu(xx):
        hh = jnp.dot(xx, w1, preferred_element_type=jnp.float32)
        a = hh[:, :D]
        return a + a * jnp.tanh(hh[:, D:])

    h_ref[8:8 + TT, :] = glu(x_ref[0])
    hn = glu(xn_ref[0])
    h_ref[8 + TT:8 + TT + 16, :] = jnp.where(i < n - 1, hn, 0.0)
    dw = dw_ref[...].astype(jnp.float32) * 0.5
    out = h_ref[6:6 + TT, :] * dw[0:1, :]
    for k in range(1, 5):
        out = out + h_ref[6 + k:6 + k + TT, :] * dw[k:k + 1, :]
    s = (out + out * jnp.tanh(out)).astype(jnp.bfloat16)
    o_ref[0] = jnp.dot(s, w2_ref[...], preferred_element_type=jnp.float32).astype(o_ref.dtype)


@jax.jit
def pallas_standalone__conformer_conv_module__speech_kernel(
    x: jax.Array,
    w_pw1: jax.Array,
    dw: jax.Array,
    w_pw2: jax.Array,
):
    B, T, D = x.shape
    nT = T // TT
    nb16 = T // 16
    return pl.pallas_call(
        _kernel,
        grid=(B, nT),
        in_specs=[
            pl.BlockSpec((1, TT, D), lambda b, i: (b, i, 0)),
            pl.BlockSpec((1, 16, D), lambda b, i: (b, jnp.minimum((i + 1) * (TT // 16), nb16 - 1), 0)),
            pl.BlockSpec((D, 2 * D), lambda b, i: (0, 0)),
            pl.BlockSpec((5, D), lambda b, i: (0, 0)),
            pl.BlockSpec((D, D), lambda b, i: (0, 0)),
        ],
        out_specs=pl.BlockSpec((1, TT, D), lambda b, i: (b, i, 0)),
        out_shape=jax.ShapeDtypeStruct((B, T, D), x.dtype),
        scratch_shapes=[pltpu.VMEM((TT + 24, D), jnp.float32), pltpu.VMEM((D, 2 * D), jnp.bfloat16)],
        compiler_params=pltpu.CompilerParams(
            dimension_semantics=("arbitrary", "arbitrary"),
            vmem_limit_bytes=100 * 1024 * 1024),
    )(x, x, w_pw1, dw, w_pw2)
```

```python
import jax
import jax.numpy as jnp
from jax import lax
import jax.experimental.pallas as pl
import jax.experimental.pallas.tpu as pltpu

P = 5
HEAD = (400, 1200, 2400)
BIG = sum(HEAD)
OUTP = (400, 800, 800, 800, 800, 400)
HALO = 16


def _make_kernel(N, T, D):
    NB = T // BIG
    NL = (N // BIG) - 1
    NH = len(HEAD)
    NQ = D // 128
    hstart = [sum(HEAD[:i]) for i in range(NH + 1)]

    def kernel(x_hbm, w1_hbm, dw_hbm, w2_hbm, o_hbm,
               xall, xh, oall, w1v, dwv, w2v, w1s, h_ref, s_ref, carry,
               in_sem, out_sem, w_sem):

        def in_copies(slot, start, size, hst):
            return (
                pltpu.make_async_copy(x_hbm.at[pl.ds(start, size)],
                                      xall.at[pl.ds(start, size)], in_sem.at[slot]),
                pltpu.make_async_copy(x_hbm.at[pl.ds(hst, HALO)],
                                      xh.at[slot], in_sem.at[slot]),
            )

        def head_copies(c):
            size = HEAD[c] if c < NH else BIG
            return in_copies(c % 2, hstart[c], size, hstart[c] + size)

        def big_copies(k):
            st = pl.multiple_of((k + 1) * BIG, 16)
            hst = pl.multiple_of(jnp.minimum((k + 2) * BIG, N - HALO), 16)
            return in_copies((k + NH) % 2, st, BIG, hst)

        wc = [pltpu.make_async_copy(w1_hbm, w1v, w_sem.at[0]),
              pltpu.make_async_copy(dw_hbm, dwv, w_sem.at[1]),
              pltpu.make_async_copy(w2_hbm, w2v, w_sem.at[1])]

        wc[0].start()
        for cp in head_copies(0):
            cp.start()
        wc[1].start()
        wc[2].start()
        wc[0].wait()
        for cp in head_copies(1):
            cp.start()
        w1s[...] = (w1v[...].astype(jnp.float32) * 0.5).astype(jnp.bfloat16)
        wc[1].wait()
        wc[2].wait()

        def process(slot, start, C, prev_zero, next_zero, pieces):
            J = C // P
            if prev_zero is True:
                h_ref[:, 0:8, :] = jnp.zeros((NQ, 8, 128), jnp.float32)
            elif prev_zero is False:
                h_ref[:, 0:8, :] = carry[...]
            else:
                h_ref[:, 0:8, :] = jnp.where(prev_zero, 0.0, carry[...])
            xx = jnp.concatenate([xall[pl.ds(start, C), :], xh[slot]], axis=0)
            hh = jnp.dot(xx, w1s[...], preferred_element_type=jnp.float32)
            a = hh[:, :D]
            ha = a + a * jnp.tanh(hh[:, D:])
            hm = ha[:C]
            hn = ha[C:]
            if next_zero is not False:
                hn = jnp.where(next_zero, 0.0, hn)
            for q in range(NQ):
                h_ref[q, 8:8 + C, :] = hm[:, q * 128:(q + 1) * 128]
                h_ref[q, 8 + C:8 + C + HALO, :] = hn[:, q * 128:(q + 1) * 128]
            carry[...] = h_ref[:, C:C + 8, :]
            dw = dwv[...].astype(jnp.float32) * 0.5
            for q in range(NQ):
                dwc = dw[:, q * 128:(q + 1) * 128]
                hs = [h_ref[q, pl.ds(6 + r, J, stride=P), :] for r in range(P + 4)]
                for s in range(P):
                    y = hs[s] * dwc[0:1, :]
                    for k in range(1, 5):
                        y = y + hs[s + k] * dwc[k:k + 1, :]
                    s_ref[q, pl.ds(s, J, stride=P), :] = y + y * jnp.tanh(y)
            o = 0
            for S in pieces:
                sv = jnp.concatenate([s_ref[q, o:o + S, :] for q in range(NQ)],
                                     axis=1).astype(jnp.bfloat16)
                st = start + o
                if not isinstance(st, int):
                    st = pl.multiple_of(st, 16)
                oall[pl.ds(st, S), :] = jnp.dot(
                    sv, w2v[...], preferred_element_type=jnp.float32).astype(oall.dtype)
                pltpu.make_async_copy(oall.at[pl.ds(st, S)], o_hbm.at[pl.ds(st, S)],
                                      out_sem).start()
                o += S

        for c in range(NH):
            for cp in head_copies(c):
                cp.wait()
            if c >= 1:
                for cp in head_copies(c + 1):
                    cp.start()
            process(c % 2, hstart[c], HEAD[c], c == 0, False, (HEAD[c],))

        def body(k, _):
            for cp in big_copies(k):
                cp.wait()

            @pl.when(k + 1 < NL)
            def _():
                for cp in big_copies(k + 1):
                    cp.start()

            start = pl.multiple_of((k + 1) * BIG, 16)
            kb = (k + 1) % NB
            process((k + NH) % 2, start, BIG, kb == 0, kb == NB - 1, OUTP)
            return 0

        lax.fori_loop(0, NL, body, 0)
        pltpu.make_async_copy(oall, o_hbm, out_sem).wait()

    return kernel


@jax.jit
def pallas_standalone__conformer_conv_module__speech_kernel(
    x: jax.Array,
    w_pw1: jax.Array,
    dw: jax.Array,
    w_pw2: jax.Array,
):
    B, T, D = x.shape
    K = dw.shape[0]
    N = B * T
    assert K == 5 and D % 128 == 0 and T % BIG == 0 and sum(OUTP) == BIG
    assert all(v % (8 * P) == 0 and v % 16 == 0 for v in HEAD) and all(v % 16 == 0 for v in OUTP)
    NQ = D // 128
    out = pl.pallas_call(
        _make_kernel(N, T, D),
        in_specs=[pl.BlockSpec(memory_space=pl.ANY)] * 4,
        out_specs=pl.BlockSpec(memory_space=pl.ANY),
        out_shape=jax.ShapeDtypeStruct((N, D), x.dtype),
        scratch_shapes=[
            pltpu.VMEM((N, D), x.dtype),
            pltpu.VMEM((2, HALO, D), x.dtype),
            pltpu.VMEM((N, D), x.dtype),
            pltpu.VMEM((D, 2 * D), w_pw1.dtype),
            pltpu.VMEM((K, D), dw.dtype),
            pltpu.VMEM((D, D), w_pw2.dtype),
            pltpu.VMEM((D, 2 * D), jnp.bfloat16),
            pltpu.VMEM((NQ, BIG + 8 + HALO, 128), jnp.float32),
            pltpu.VMEM((NQ, BIG + 8, 128), jnp.float32),
            pltpu.VMEM((NQ, 8, 128), jnp.float32),
            pltpu.SemaphoreType.DMA((2,)),
            pltpu.SemaphoreType.DMA(()),
            pltpu.SemaphoreType.DMA((2,)),
        ],
        compiler_params=pltpu.CompilerParams(
            vmem_limit_bytes=100 * 1024 * 1024,
            disable_bounds_checks=True),
    )(x.reshape(N, D), w_pw1, dw, w_pw2)
    return out.reshape(B, T, D)
```
